```python
import os as _os
_os.environ.setdefault("JAX_PLATFORMS", "cpu")
import jax
import jax.numpy as jnp

def _softmax(x, axis=-1):
    return jax.nn.softmax(x, axis=axis)
def _gelu(x):
    return jax.nn.gelu(x, approximate=True)
def _silu(x):
    return jax.nn.silu(x)
def _sigmoid(x):
    return jax.nn.sigmoid(x)
def _layernorm(x, axis=-1, eps=1e-5):
    m = jnp.mean(x, axis=axis, keepdims=True)
    v = jnp.var(x, axis=axis, keepdims=True)
    return (x - m) / jnp.sqrt(v + eps)
def _scatter_add(tgt, idx, src, axis=0):
    return tgt.at[idx].add(src)
def _segment_sum(src, seg, n):
    return jax.ops.segment_sum(src, seg, n)
class _Rng:
    def __init__(self, key):
        self._k = key
    def _next(self):
        self._k, sub = jax.random.split(self._k)
        return sub
    def normal(self, shape):
        return jax.random.normal(self._next(), shape, dtype=jnp.bfloat16)
    def randint(self, lo, hi, shape):
        return jax.random.randint(self._next(), shape, lo, hi, dtype=jnp.int32)
    def uniform(self, shape, lo=0.0, hi=1.0):
        return jax.random.uniform(self._next(), shape, jnp.bfloat16, lo, hi)
    def permutation(self, n):
        return jax.random.permutation(self._next(), n)


kernel_name = 'gated_mix__softmax_full_mha__spectral_gfnet__prompt'

def setup_inputs():
    _rng = _Rng(jax.random.key(int.from_bytes(__import__("os").urandom(4), "little")))
    _w = (lambda a: (lambda t: t.astype(jnp.bfloat16) if jnp.issubdtype(t.dtype, jnp.floating) else t)(jnp.asarray(a)))
    def _A_setup():
        B, S, D = 1, 2048, 448
        return {
            "x": _w((lambda *s: _rng.normal(s) * 0.05)(B, S, D)),
            "wqkv": _w((lambda *s: _rng.normal(s) * 0.4)(D, 3 * D)),
            "wo": _w((lambda *s: _rng.normal(s) * 0.05)(D, D)),
        }
    _A_in = _A_setup()

    def _B_setup():
        B, S, D = 1, 2048, 448
        Df = D // 2 + 1
        return {
            "x": _w((lambda *s: _rng.normal(s) * 0.05)(B, S, D)),
            "w_r": _w((lambda *s: _rng.normal(s) * 1.6)(S, Df) * 0.02),
            "w_i": _w((lambda *s: _rng.normal(s) * 1.6)(S, Df) * 0.02),
        }
    _B_in = _B_setup()

    return {
        "A_x": _A_in["x"],
        "A_wqkv": _A_in["wqkv"],
        "A_wo": _A_in["wo"],
        "B_x": _B_in["x"],
        "B_w_r": _B_in["w_r"],
        "B_w_i": _B_in["w_i"],
        "gate_w": _w((lambda *s: _rng.normal(s) * 0.05)(448) * 16.0),
    }

def reference(A_x, A_wqkv, A_wo, B_x, B_w_r, B_w_i, gate_w):
    def _A_ref(x, wqkv, wo):
        B, S, D = x.shape
        H = 16; Dh = D // H
        qkv = (lambda x, *d: x.transpose(*d))((x @ wqkv).reshape(B, S, 3, H, Dh), 2, 0, 3, 1, 4)
        q, k, v = qkv[0], qkv[1], qkv[2]
        scale = Dh ** -0.5
        scores = jnp.einsum("bhqd,bhkd->bhqk", q, k) * scale
        p = _softmax(scores, axis=-1)
        o = jnp.einsum("bhqk,bhkd->bhqd", p, v)
        return (lambda x, *d: x.transpose(*d))(o, 0, 2, 1, 3).reshape(B, S, D) @ wo

    def _B_ref(x, w_r, w_i):
        B, S, D = x.shape
        X = (lambda x, axes=(-2,-1): jnp.fft.rfft2(x.astype(jnp.float32), axes=axes))(x, axes=(-2, -1))
        W = w_r + 1j * w_i
        X = X * W
        y = (lambda x, s, axes=(-2,-1): jnp.fft.irfft2(x, s=s, axes=axes).astype(jnp.bfloat16))(X, (S, D), axes=(-2, -1))
        return y

    x = A_x
    g = _sigmoid((x * gate_w).sum(-1, keepdims=True))
    a = _A_ref(x, A_wqkv, A_wo)
    b = _B_ref(x, B_w_r, B_w_i)
    return g * a + (1 - g) * b
```

```python
import functools

import numpy as np
import jax
import jax.numpy as jnp
from jax import lax
import jax.experimental.pallas as pl
import jax.experimental.pallas.tpu as pltpu

F32 = jnp.float32
BF16 = jnp.bfloat16
U32 = jnp.uint32

S, D, H, DH = 2048, 448, 16, 28
DF = D // 2 + 1
Q4 = D // 4
QB = 512
NQB = S // QB
AW = 1024
NAQ = S // AW
NBLK = H * NAQ
NIT = NBLK // 2 - 1
GPI = 2

_CLASS_ORDER = (0, 2, 1, 3)
_CLASS_GROUPS = {0: 8, 2: 7, 1: 7, 3: 7}
_GROUPS = [(r, g) for r in _CLASS_ORDER for g in range(_CLASS_GROUPS[r])]
NG = len(_GROUPS)
NROW = 16 * NG

_O_FF, _O_CF, _O_CI = 0, NROW, NROW + 256
_O_G0 = _O_CI + 256
_O_G2 = _O_G0 + Q4
_O_GAB = _O_G2 + Q4
_CB_ROWS = _O_GAB + 2 * Q4


def _pack_rows_np(a):
    u = np.ascontiguousarray(a, dtype=np.float32).view(np.uint32)
    b = ((u + 0x7FFF + ((u >> 16) & 1)) >> 16).astype(np.uint32)
    return b[0::2] | (b[1::2] << 16)


@functools.lru_cache(maxsize=1)
def _tables():
    rows = []
    for (r, g) in _GROUPS:
        for part in (0, 1):
            for i in range(8):
                rows.append((r + 4 * (8 * g + i), part))
    dp = np.arange(Q4)
    cb = np.zeros((_CB_ROWS, 256), np.float64)
    norm = 1.0 / (S * D)
    for row, (f, im) in enumerate(rows):
        if f > D // 2:
            continue
        r = f % 4
        th = 2 * np.pi * f * dp / D
        c, s = np.cos(th), np.sin(th)
        if r in (0, 2):
            cb[_O_FF + row, :Q4] = -s if im else c
        elif r == 1:
            cb[_O_FF + row, :Q4] = -s if im else c
            cb[_O_FF + row, 128:128 + Q4] = -c if im else -s
        else:
            cb[_O_FF + row, :Q4] = -s if im else c
            cb[_O_FF + row, 128:128 + Q4] = c if im else s
        cf = (1.0 if f in (0, D // 2) else 2.0) * norm
        re_part = (-s if im else c) * cf
        im_part = (c if im else s) * cf
        if r == 0:
            cb[_O_G0:_O_G0 + Q4, row] = re_part
        elif r == 2:
            cb[_O_G2:_O_G2 + Q4, row - 128] = re_part
        else:
            cb[_O_GAB:_O_GAB + Q4, row - 240] = re_part
            cb[_O_GAB + Q4:_O_GAB + 2 * Q4, row - 240] = -im_part if r == 1 else im_part
    b = np.arange(128)
    ph = 2 * np.pi * np.outer(b, b) / 128
    c, s = np.cos(ph), np.sin(ph)
    k2 = 8 * (b % 16) + b // 16
    cf_, sf_ = c[:, k2], s[:, k2]
    cb[_O_CF:_O_CF + 256] = np.block([[cf_, -sf_], [sf_, cf_]])
    cb[_O_CI:_O_CI + 256] = np.block([[cf_.T, sf_.T], [-sf_.T, cf_.T]])
    tw = 2 * np.pi * np.outer(np.arange(16), b) / S
    twid = np.concatenate([np.repeat(np.cos(tw), 8, axis=0), np.repeat(np.sin(tw), 8, axis=0)], 0)
    return _pack_rows_np(cb), twid.astype(np.float32)


def _pk(x):
    return pltpu.bitcast(x, U32)


def _upk(x):
    return pltpu.bitcast(x, BF16)


def _dot(a, b):
    return jnp.dot(a, b, preferred_element_type=F32)


def _dot_nt(a, b):
    return lax.dot_general(a, b, (((1,), (1,)), ((), ())), preferred_element_type=F32)


def _cmul_const(z, ang):
    re, im = z
    k = int(round(ang / (2 * np.pi / 16))) % 16
    if k == 0:
        return z
    if k == 4:
        return (-im, re)
    if k == 8:
        return (-re, -im)
    if k == 12:
        return (im, -re)
    c, s = float(np.cos(ang)), float(np.sin(ang))
    if k % 4 == 2:
        a = abs(c)
        p, m = (re + im) * a, (re - im) * a
        if k == 2:
            return (m, p)
        if k == 6:
            return (-p, m)
        if k == 10:
            return (-m, -p)
        return (p, -m)
    return (re * c - im * s, re * s + im * c)


def _dft4(x, sign):
    (r0, i0), (r1, i1), (r2, i2), (r3, i3) = x
    ar, ai = r0 + r2, i0 + i2
    br, bi = r0 - r2, i0 - i2
    cr, ci = r1 + r3, i1 + i3
    dr, di = r1 - r3, i1 - i3
    y0 = (ar + cr, ai + ci)
    y2 = (ar - cr, ai - ci)
    ym = (br + di, bi - dr)
    yp = (br - di, bi + dr)
    return [y0, ym, y2, yp] if sign < 0 else [y0, yp, y2, ym]


def _dft16(x, sign):
    a = [_dft4([x[4 * n1 + n0] for n1 in range(4)], sign) for n0 in range(4)]
    out = [None] * 16
    for k0 in range(4):
        col = [_cmul_const(a[n0][k0], sign * 2 * np.pi * n0 * k0 / 16) for n0 in range(4)]
        y = _dft4(col, sign)
        for k1 in range(4):
            out[k0 + 4 * k1] = y[k1]
    return out


_SAFE_SCORE = 60.0
_V_HI = 2.0 ** 50
_V_LO = 2.0 ** -40


def _kernel(xt_hbm, wqkv_hbm, wo_hbm, wr_hbm, wi_hbm, gate_hbm, cb_hbm, tw_hbm, out_hbm,
            xs, wq_s, wo_s, wr_s, wi_s, gate_s, cb, tw,
            lhs_all, wot, ks, qt, vt, ot, gt,
            p0, p1, x1t, w32, zt, outb, sbuf,
            sem_x, sem_w, sem_in, sem_out):
    def x_copy(b):
        c = pl.ds(pl.multiple_of(b * QB, QB), QB)
        return pltpu.make_async_copy(xt_hbm.at[:, c], xs.at[:, c], sem_x.at[b])

    w_chunks = [(0, 128), (128, 128), (256, 128), (384, 64)]
    w_copies = [pltpu.make_async_copy(wqkv_hbm.at[pl.ds(o, n), :], wq_s.at[pl.ds(o, n), :], sem_w.at[i])
                for i, (o, n) in enumerate(w_chunks)]
    in_copies = [
        pltpu.make_async_copy(src, dst, sem_in.at[i])
        for i, (src, dst) in enumerate([(gate_hbm, gate_s), (cb_hbm, cb), (tw_hbm, tw),
                                        (wo_hbm, wo_s), (wr_hbm, wr_s), (wi_hbm, wi_s)])]
    for c in w_copies:
        c.start()
    in_copies[0].start()
    x_copy(0).start()

    def cbt(off, rows, lo, hi):
        return _upk(cb[off // 2:(off + rows) // 2, :])[:, lo:hi]

    for i, (o, n) in enumerate(w_chunks):
        w_copies[i].wait()
        if i == len(w_chunks) - 1:
            for b in range(1, NQB):
                x_copy(b).start()
        lhs_all[0:3 * D // 2, o:o + n] = _pk(wq_s[o:o + n, :].T)
    in_copies[0].wait()
    gate16 = jnp.concatenate([gate_s[...].reshape(1, D).astype(F32), jnp.zeros((15, D), F32)], axis=0)
    lhs_all[3 * D // 2:3 * D // 2 + 8, :] = _pk(gate16.astype(BF16))

    qscale = float(DH ** -0.5 * np.log2(np.e))

    def lane_tile_max(a):
        parts = [a[:, 128 * j:128 * j + 128] for j in range(a.shape[1] // 128)]
        while len(parts) > 1:
            parts = [jnp.maximum(parts[i], parts[i + 1]) if i + 1 < len(parts) else parts[i]
                     for i in range(0, len(parts), 2)]
        return parts[0]

    def proj_block(c0, n):
        xb = xs[:, c0:c0 + n]
        qkv = _dot(_upk(lhs_all[...]), xb)
        q = (qkv[0:D] * qscale).astype(BF16)
        qt[:, c0:c0 + n] = _pk(q)
        amax = lane_tile_max(jnp.abs(q.astype(F32)))
        k = qkv[D:2 * D].astype(BF16)
        kmax = lane_tile_max(jnp.abs(k.astype(F32)))
        for t in range(4):
            kg = jnp.concatenate([k[Q4 * t:Q4 * t + Q4], jnp.zeros((16, n), BF16)], axis=0)
            ks[c0 // 2:(c0 + n) // 2, 128 * t:128 * t + 128] = _pk(kg.T)
        v = qkv[2 * D:3 * D]
        vmax = lane_tile_max(jnp.max(jnp.abs(v).reshape(D // 8, 8, n), axis=0))
        tail = (lax.broadcasted_iota(jnp.int32, (4, n), 0) == 0).astype(F32)
        parts = []
        for h in range(H):
            parts += [v[DH * h:DH * h + DH], tail]
        vt[:, c0:c0 + n] = _pk(jnp.concatenate(parts, axis=0).astype(BF16))
        gt[:, c0:c0 + n] = jnp.broadcast_to(qkv[3 * D:3 * D + 1], (8, n))
        return amax, kmax, vmax

    x_copy(0).wait()
    st = [proj_block(0, QB)]
    for c in in_copies[1:]:
        c.start()
    for b in range(1, NQB):
        x_copy(b).wait()
    for b in range(1, NQB):
        st.append(proj_block(b * QB, QB))
    amax, kmax, vmax = [jnp.maximum(jnp.maximum(a, b), jnp.maximum(c, d)) for a, b, c, d in zip(*st)]

    kcol = jnp.max(kmax, axis=1, keepdims=True)
    prod = (amax * kcol).astype(BF16)
    hh = lax.broadcasted_iota(jnp.int32, (H, D), 0)
    jj = lax.broadcasted_iota(jnp.int32, (H, D), 1)
    ind = jnp.where((jj >= DH * hh) & (jj < DH * hh + DH), 1.0, 0.0).astype(BF16)
    bound = jnp.max(_dot(ind, prod)) * 1.03
    vmax = jnp.max(vmax)
    safe = jnp.logical_and(bound <= _SAFE_SCORE, jnp.logical_and(vmax <= _V_HI, vmax >= _V_LO))

    in_copies[1].wait()
    for b in range(NQB):
        cols = slice(b * QB, (b + 1) * QB)
        xf = xs[:, cols].astype(F32)
        x0, x1, x2, x3 = [xf[Q4 * j:Q4 * j + Q4] for j in range(4)]
        sa, sb = x0 + x2, x1 + x3
        y0 = (sa + sb).astype(BF16)
        y2 = (sa - sb).astype(BF16)
        u = (x0 - x2).astype(BF16)
        w = (x1 - x3).astype(BF16)
        x1t[0:128, cols] = _dot(cbt(_O_FF, 128, 0, Q4), y0)
        x1t[128:240, cols] = _dot(cbt(_O_FF + 128, Q4, 0, Q4), y2)
        x1t[240:464, cols] = (_dot(cbt(_O_FF + 240, 224, 0, Q4), u)
                              + _dot(cbt(_O_FF + 240, 224, 128, 128 + Q4), w))

    for c in in_copies[2:]:
        c.wait()

    def late_prep():
        for a, w_s in enumerate((wr_s, wi_s)):
            last = jnp.concatenate([w_s[DF - 1:DF, :].astype(F32), jnp.zeros((31, S), F32)], axis=0).astype(BF16)
            for j in range(16):
                w32[a, j, 0:112, :] = _pk(w_s[0:DF - 1, 128 * j:128 * j + 128])
                w32[a, j, 112:128, :] = _pk(last[:, 128 * j:128 * j + 128])
        wo = wo_s[...].astype(F32)
        parts = []
        for h in range(H):
            parts += [wo[DH * h:DH * h + DH], jnp.zeros((4, D), F32)]
        wot[...] = _pk(jnp.concatenate(parts, axis=0).astype(BF16).T)

    def tw_pair(k1):
        return tw[8 * k1:8 * k1 + 8, :], tw[128 + 8 * k1:128 + 8 * k1 + 8, :]

    def fft_a1(gi):
        rows = pl.ds(pl.multiple_of(gi * 16, 16), 16)
        blk = x1t[rows, :]
        xin = [(blk[0:8, 128 * a:128 * a + 128], blk[8:16, 128 * a:128 * a + 128]) for a in range(16)]
        y = _dft16(xin, -1)
        out = []
        for k1 in range(16):
            re, im = y[k1]
            if k1:
                c, s = tw_pair(k1)
                re, im = re * c + im * s, im * c - re * s
            out.append(jnp.concatenate([re, im], axis=1))
        return jnp.concatenate(out, axis=0).astype(BF16)

    def fft_a(gis):
        return jnp.concatenate([fft_a1(gi) for gi in gis], axis=0)

    def filter_rows(a, p_start, shift):
        v = []
        for j in range(16):
            w = w32[a, j, pl.ds(p_start, 8, stride=2), :]
            v.append(pltpu.bitcast((w << shift) & jnp.uint32(0xFFFF0000), F32))
        lane = lax.broadcasted_iota(jnp.int32, (8, 128), 1)
        for i in range(4):
            d = 1 << i
            low = (lane & d) == 0
            for j in range(16):
                if j & d == 0:
                    lo, hi = v[j], v[j + d]
                    v[j] = jnp.where(low, lo, pltpu.roll(hi, d, 1))
                    v[j + d] = jnp.where(low, pltpu.roll(lo, 128 - d, 1), hi)
        return v

    def fft_b(gis, l1):
        xf_all = _dot(l1, cbt(_O_CF, 256, 0, 256))
        out = []
        for n, gi in enumerate(gis):
            r = jnp.where(gi < 8, 0, jnp.where(gi < 15, 2, jnp.where(gi < 22, 1, 3)))
            g = gi - jnp.where(gi < 8, 0, jnp.where(gi < 15, 8, jnp.where(gi < 22, 15, 22)))
            p_start = r // 2 + 16 * g
            shift = jnp.asarray(16 - 16 * (r % 2)).astype(U32)
            wr_ = filter_rows(0, p_start, shift)
            wi_ = filter_rows(1, p_start, shift)
            xf = xf_all[128 * n:128 * n + 128]
            for k1 in range(16):
                re, im = xf[8 * k1:8 * k1 + 8, 0:128], xf[8 * k1:8 * k1 + 8, 128:256]
                out.append(jnp.concatenate([re * wr_[k1] - im * wi_[k1], re * wi_[k1] + im * wr_[k1]], axis=1))
        return jnp.concatenate(out, axis=0).astype(BF16)

    def fft_c(gis, l2):
        zf_all = _dot(l2, cbt(_O_CI, 256, 0, 256))
        for n, gi in enumerate(gis):
            zf = zf_all[128 * n:128 * n + 128]
            xin = []
            for k1 in range(16):
                re, im = zf[8 * k1:8 * k1 + 8, 0:128], zf[8 * k1:8 * k1 + 8, 128:256]
                if k1:
                    c, s = tw_pair(k1)
                    re, im = re * c - im * s, im * c + re * s
                xin.append((re, im))
            z = _dft16(xin, +1)
            top = jnp.concatenate([z[a][0] for a in range(16)], axis=1)
            bot = jnp.concatenate([z[a][1] for a in range(16)], axis=1)
            zt[pl.ds(pl.multiple_of(gi * 8, 8), 8), :] = _pk(jnp.concatenate([top, bot], axis=0).astype(BF16))

    def scores(n):
        h = n // NAQ
        t = h // 4
        i = h % 4
        cols = pl.ds(pl.multiple_of((n % NAQ) * AW, AW), AW)
        q32 = qt[pl.ds(pl.multiple_of(56 * t, 8), 56), cols]
        rr = lax.broadcasted_iota(jnp.int32, (56, AW), 0)
        q32 = jnp.where((rr >= 14 * i) & (rr < 14 * i + 14), q32, jnp.uint32(0))
        qm = _upk(jnp.concatenate([q32, jnp.zeros((8, AW), U32)], axis=0))
        kt = _upk(ks[:, pl.ds(pl.multiple_of(128 * t, 128), 128)])
        return _dot(kt, qm)

    def qk_exp(n, p_ref):
        p_ref[...] = _pk(jnp.exp2(scores(n)).astype(BF16))

    def pv(n, p_ref):
        h = n // NAQ
        rows = pl.ds(pl.multiple_of(16 * h, 16), 16)
        o = _dot(_upk(vt[rows, :]), _upk(p_ref[...]))
        o = o * (1.0 / o[DH:DH + 1, :])
        ot[rows, pl.ds(pl.multiple_of((n % NAQ) * AW, AW), AW)] = _pk(o.astype(BF16))

    @pl.when(safe)
    def _fast():
        late_prep()
        qk_exp(0, p0)

        def body(j, carry):
            gis = [jnp.minimum(GPI * j + m, NG - 1) for m in range(GPI)]
            l1 = fft_a(gis)
            qk_exp(2 * j + 1, p1)
            l2 = fft_b(gis, l1)
            pv(2 * j, p0)
            qk_exp(2 * j + 2, p0)
            fft_c(gis, l2)
            pv(2 * j + 1, p1)
            return carry

        lax.fori_loop(0, NIT, body, 0)
        gis = list(range(NIT * GPI, NG))
        if gis:
            l1 = fft_a(gis)
        qk_exp(NBLK - 1, p1)
        if gis:
            l2 = fft_b(gis, l1)
        pv(NBLK - 2, p0)
        if gis:
            fft_c(gis, l2)
        pv(NBLK - 1, p1)

    @pl.when(jnp.logical_not(safe))
    def _slow():
        late_prep()

        def body(n, carry):
            sbuf[...] = scores(n)
            m = jnp.max(jnp.max(sbuf[...].reshape(S // 8, 8, AW), axis=0), axis=0, keepdims=True)
            p0[...] = _pk(jnp.exp2(sbuf[...] - m).astype(BF16))
            pv(n, p0)
            return carry

        lax.fori_loop(0, NBLK, body, 0)

        def fbody(gi, carry):
            fft_c([gi], fft_b([gi], fft_a([gi])))
            return carry

        lax.fori_loop(0, NG, fbody, 0)

    def out_copy(b):
        c = pl.ds(pl.multiple_of(b * QB, QB), QB)
        return pltpu.make_async_copy(outb.at[:, c], out_hbm.at[:, c], sem_out.at[b])

    def final_block(b, carry):
        cols = pl.ds(b * QB, QB)
        at = _dot(_upk(wot[...]), _upk(ot[:, cols]))
        t0 = _dot(cbt(_O_G0, Q4, 0, 128), _upk(zt[0:64, cols]))
        t2 = _dot(cbt(_O_G2, Q4, 0, Q4), _upk(zt[64:120, cols]))
        ab = _dot(cbt(_O_GAB, 2 * Q4, 0, 2 * Q4), _upk(zt[120:232, cols]))
        e, o = t0 + t2, t0 - t2
        yt = jnp.concatenate([e + ab[0:Q4], o + ab[Q4:], e - ab[0:Q4], o - ab[Q4:]], axis=0)
        g = jax.nn.sigmoid(gt[0:1, cols])
        outb[:, cols] = (g * at + (1.0 - g) * yt).astype(BF16)
        out_copy(b).start()
        return carry

    for b in range(NQB):
        final_block(b, 0)
    for b in range(NQB):
        out_copy(b).wait()


@jax.jit
def pallas_gated_mix__softmax_full_mha__spectral_gfnet__prompt_kernel(
    A_x: jax.Array,
    A_wqkv: jax.Array,
    A_wo: jax.Array,
    B_x: jax.Array,
    B_w_r: jax.Array,
    B_w_i: jax.Array,
    gate_w: jax.Array,
):
    del B_x
    cb_np, tw_np = _tables()
    any_spec = pl.BlockSpec(memory_space=pltpu.HBM)
    scratch = [
        pltpu.VMEM((D, S), BF16),
        pltpu.VMEM((D, 3 * D), BF16),
        pltpu.VMEM((D, D), BF16),
        pltpu.VMEM((DF, S), BF16),
        pltpu.VMEM((DF, S), BF16),
        pltpu.VMEM((D,), BF16),
        pltpu.VMEM(cb_np.shape, U32),
        pltpu.VMEM(tw_np.shape, F32),
        pltpu.VMEM((3 * D // 2 + 8, D), U32),
        pltpu.VMEM((D // 2, 512), U32),
        pltpu.VMEM((S // 2, 512), U32),
        pltpu.VMEM((D // 2, S), U32),
        pltpu.VMEM((256, S), U32),
        pltpu.VMEM((256, S), U32),
        pltpu.VMEM((8, S), F32),
        pltpu.VMEM((S // 2, AW), U32),
        pltpu.VMEM((S // 2, AW), U32),
        pltpu.VMEM((NROW, S), F32),
        pltpu.VMEM((2, 16, 128, 128), U32),
        pltpu.VMEM((NROW // 2, S), U32),
        pltpu.VMEM((D, S), BF16),
        pltpu.VMEM((S, AW), F32),
        pltpu.SemaphoreType.DMA((NQB,)),
        pltpu.SemaphoreType.DMA((4,)),
        pltpu.SemaphoreType.DMA((6,)),
        pltpu.SemaphoreType.DMA((NQB,)),
    ]
    out = pl.pallas_call(
        _kernel,
        out_shape=jax.ShapeDtypeStruct((D, S), BF16),
        in_specs=[any_spec] * 8,
        out_specs=any_spec,
        scratch_shapes=scratch,
        compiler_params=pltpu.CompilerParams(vmem_limit_bytes=100 * 1024 * 1024),
    )(A_x.reshape(S, D).T, A_wqkv, A_wo, B_w_r.T, B_w_i.T, gate_w, jnp.asarray(cb_np), jnp.asarray(tw_np))
    return out.T.reshape(1, S, D)
```

```python
import functools

import numpy as np
import jax
import jax.numpy as jnp
from jax import lax
import jax.experimental.pallas as pl
import jax.experimental.pallas.tpu as pltpu

F32 = jnp.float32
BF16 = jnp.bfloat16
U32 = jnp.uint32

S, D, H, DH = 2048, 448, 16, 28
DF = D // 2 + 1
Q4 = D // 4
QB = 512
NQB = S // QB
AW = 1024
NAQ = S // AW
NBLK = H * NAQ
NIT = NBLK // 2 - 1
GPI = 2

_CLASS_ORDER = (0, 2, 1, 3)
_CLASS_GROUPS = {0: 8, 2: 7, 1: 7, 3: 7}
_GROUPS = [(r, g) for r in _CLASS_ORDER for g in range(_CLASS_GROUPS[r])]
NG = len(_GROUPS)
NROW = 16 * NG

_O_FF = 0
_O_G0 = NROW
_O_G2 = _O_G0 + Q4
_O_GAB = _O_G2 + Q4
_CB_ROWS = _O_GAB + 2 * Q4


def _pack_rows_np(a):
    u = np.ascontiguousarray(a, dtype=np.float32).view(np.uint32)
    b = ((u + 0x7FFF + ((u >> 16) & 1)) >> 16).astype(np.uint32)
    return b[0::2] | (b[1::2] << 16)


@functools.lru_cache(maxsize=1)
def _tables():
    rows = []
    for (r, g) in _GROUPS:
        for part in (0, 1):
            for i in range(8):
                rows.append((r + 4 * (8 * g + i), part))
    dp = np.arange(Q4)
    cb = np.zeros((_CB_ROWS, 256), np.float64)
    norm = 1.0 / (S * D)
    for row, (f, im) in enumerate(rows):
        if f > D // 2:
            continue
        r = f % 4
        th = 2 * np.pi * f * dp / D
        c, s = np.cos(th), np.sin(th)
        if r in (0, 2):
            cb[_O_FF + row, :Q4] = -s if im else c
        elif r == 1:
            cb[_O_FF + row, :Q4] = -s if im else c
            cb[_O_FF + row, 128:128 + Q4] = -c if im else -s
        else:
            cb[_O_FF + row, :Q4] = -s if im else c
            cb[_O_FF + row, 128:128 + Q4] = c if im else s
        cf = (1.0 if f in (0, D // 2) else 2.0) * norm
        re_part = (-s if im else c) * cf
        im_part = (c if im else s) * cf
        if r == 0:
            cb[_O_G0:_O_G0 + Q4, row] = re_part
        elif r == 2:
            cb[_O_G2:_O_G2 + Q4, row - 128] = re_part
        else:
            cb[_O_GAB:_O_GAB + Q4, row - 240] = re_part
            cb[_O_GAB + Q4:_O_GAB + 2 * Q4, row - 240] = -im_part if r == 1 else im_part
    b = np.arange(128)
    tw = 2 * np.pi * np.outer(np.arange(16), b) / S
    rows_tw = [np.repeat(np.cos(tw), 8, axis=0), np.repeat(np.sin(tw), 8, axis=0)]
    for h in (64, 16, 4):
        ang = 2 * np.pi * (b % (h // 2)) * (((b & h) != 0) * 1 + ((b & (h // 2)) != 0) * 2) / (2 * h)
        rows_tw += [np.repeat(np.cos(ang)[None], 8, axis=0), np.repeat(np.sin(ang)[None], 8, axis=0)]
    twid = np.concatenate(rows_tw, 0)
    return _pack_rows_np(cb), twid.astype(np.float32)


def _pk(x):
    return pltpu.bitcast(x, U32)


def _upk(x):
    return pltpu.bitcast(x, BF16)


def _dot(a, b):
    return jnp.dot(a, b, preferred_element_type=F32)


def _dot_nt(a, b):
    return lax.dot_general(a, b, (((1,), (1,)), ((), ())), preferred_element_type=F32)


def _cmul_const(z, ang):
    re, im = z
    k = int(round(ang / (2 * np.pi / 16))) % 16
    if k == 0:
        return z
    if k == 4:
        return (-im, re)
    if k == 8:
        return (-re, -im)
    if k == 12:
        return (im, -re)
    c, s = float(np.cos(ang)), float(np.sin(ang))
    if k % 4 == 2:
        a = abs(c)
        p, m = (re + im) * a, (re - im) * a
        if k == 2:
            return (m, p)
        if k == 6:
            return (-p, m)
        if k == 10:
            return (-m, -p)
        return (p, -m)
    return (re * c - im * s, re * s + im * c)


def _dft4(x, sign):
    (r0, i0), (r1, i1), (r2, i2), (r3, i3) = x
    ar, ai = r0 + r2, i0 + i2
    br, bi = r0 - r2, i0 - i2
    cr, ci = r1 + r3, i1 + i3
    dr, di = r1 - r3, i1 - i3
    y0 = (ar + cr, ai + ci)
    y2 = (ar - cr, ai - ci)
    ym = (br + di, bi - dr)
    yp = (br - di, bi + dr)
    return [y0, ym, y2, yp] if sign < 0 else [y0, yp, y2, ym]


def _dft16(x, sign):
    a = [_dft4([x[4 * n1 + n0] for n1 in range(4)], sign) for n0 in range(4)]
    out = [None] * 16
    for k0 in range(4):
        col = [_cmul_const(a[n0][k0], sign * 2 * np.pi * n0 * k0 / 16) for n0 in range(4)]
        y = _dft4(col, sign)
        for k1 in range(4):
            out[k0 + 4 * k1] = y[k1]
    return out


_SAFE_SCORE = 60.0
_V_HI = 2.0 ** 50
_V_LO = 2.0 ** -40


def _kernel(xt_hbm, wqkv_hbm, wo_hbm, wr_hbm, wi_hbm, gate_hbm, cb_hbm, tw_hbm, out_hbm,
            xs, wq_s, wo_s, wr_s, wi_s, gate_s, cb, tw,
            lhs_all, wot, ks, qt, vt, ot, gt,
            p0, p1, x1t, w32, zt, outb, sbuf,
            sem_x, sem_w, sem_in, sem_out):
    def x_copy(b):
        c = pl.ds(pl.multiple_of(b * QB, QB), QB)
        return pltpu.make_async_copy(xt_hbm.at[:, c], xs.at[:, c], sem_x.at[b])

    w_chunks = [(0, 128), (128, 128), (256, 128), (384, 64)]
    w_copies = [pltpu.make_async_copy(wqkv_hbm.at[pl.ds(o, n), :], wq_s.at[pl.ds(o, n), :], sem_w.at[i])
                for i, (o, n) in enumerate(w_chunks)]
    in_copies = [
        pltpu.make_async_copy(src, dst, sem_in.at[i])
        for i, (src, dst) in enumerate([(gate_hbm, gate_s), (cb_hbm, cb), (tw_hbm, tw),
                                        (wo_hbm, wo_s), (wr_hbm, wr_s), (wi_hbm, wi_s)])]
    for c in w_copies:
        c.start()
    in_copies[0].start()
    x_copy(0).start()

    def cbt(off, rows, lo, hi):
        return _upk(cb[off // 2:(off + rows) // 2, :])[:, lo:hi]

    for i, (o, n) in enumerate(w_chunks):
        w_copies[i].wait()
        if i == len(w_chunks) - 1:
            for b in range(1, NQB):
                x_copy(b).start()
        lhs_all[0:3 * D // 2, o:o + n] = _pk(wq_s[o:o + n, :].T)
    in_copies[0].wait()
    gate16 = jnp.concatenate([gate_s[...].reshape(1, D).astype(F32), jnp.zeros((15, D), F32)], axis=0)
    lhs_all[3 * D // 2:3 * D // 2 + 8, :] = _pk(gate16.astype(BF16))

    qscale = float(DH ** -0.5 * np.log2(np.e))

    def lane_tile_max(a):
        parts = [a[:, 128 * j:128 * j + 128] for j in range(a.shape[1] // 128)]
        while len(parts) > 1:
            parts = [jnp.maximum(parts[i], parts[i + 1]) if i + 1 < len(parts) else parts[i]
                     for i in range(0, len(parts), 2)]
        return parts[0]

    def proj_block(c0, n):
        xb = xs[:, c0:c0 + n]
        qkv = _dot(_upk(lhs_all[...]), xb)
        q = (qkv[0:D] * qscale).astype(BF16)
        qt[:, c0:c0 + n] = _pk(q)
        amax = lane_tile_max(jnp.abs(q.astype(F32)))
        k = qkv[D:2 * D].astype(BF16)
        kmax = lane_tile_max(jnp.abs(k.astype(F32)))
        for t in range(4):
            kg = jnp.concatenate([k[Q4 * t:Q4 * t + Q4], jnp.zeros((16, n), BF16)], axis=0)
            ks[c0 // 2:(c0 + n) // 2, 128 * t:128 * t + 128] = _pk(kg.T)
        v = qkv[2 * D:3 * D]
        vmax = lane_tile_max(jnp.max(jnp.abs(v).reshape(D // 8, 8, n), axis=0))
        tail = (lax.broadcasted_iota(jnp.int32, (4, n), 0) == 0).astype(F32)
        parts = []
        for h in range(H):
            parts += [v[DH * h:DH * h + DH], tail]
        vt[:, c0:c0 + n] = _pk(jnp.concatenate(parts, axis=0).astype(BF16))
        gt[:, c0:c0 + n] = jnp.broadcast_to(qkv[3 * D:3 * D + 1], (8, n))
        return amax, kmax, vmax

    x_copy(0).wait()
    st = [proj_block(0, QB)]
    for c in in_copies[1:]:
        c.start()
    for b in range(1, NQB):
        x_copy(b).wait()
    for b in range(1, NQB):
        st.append(proj_block(b * QB, QB))
    amax, kmax, vmax = [jnp.maximum(jnp.maximum(a, b), jnp.maximum(c, d)) for a, b, c, d in zip(*st)]

    kcol = jnp.max(kmax, axis=1, keepdims=True)
    prod = (amax * kcol).astype(BF16)
    hh = lax.broadcasted_iota(jnp.int32, (H, D), 0)
    jj = lax.broadcasted_iota(jnp.int32, (H, D), 1)
    ind = jnp.where((jj >= DH * hh) & (jj < DH * hh + DH), 1.0, 0.0).astype(BF16)
    bound = jnp.max(_dot(ind, prod)) * 1.03
    vmax = jnp.max(vmax)
    safe = jnp.logical_and(bound <= _SAFE_SCORE, jnp.logical_and(vmax <= _V_HI, vmax >= _V_LO))

    in_copies[1].wait()
    for b in range(NQB):
        cols = slice(b * QB, (b + 1) * QB)
        xf = xs[:, cols].astype(F32)
        x0, x1, x2, x3 = [xf[Q4 * j:Q4 * j + Q4] for j in range(4)]
        sa, sb = x0 + x2, x1 + x3
        y0 = (sa + sb).astype(BF16)
        y2 = (sa - sb).astype(BF16)
        u = (x0 - x2).astype(BF16)
        w = (x1 - x3).astype(BF16)
        x1t[0:128, cols] = _dot(cbt(_O_FF, 128, 0, Q4), y0)
        x1t[128:240, cols] = _dot(cbt(_O_FF + 128, Q4, 0, Q4), y2)
        x1t[240:464, cols] = (_dot(cbt(_O_FF + 240, 224, 0, Q4), u)
                              + _dot(cbt(_O_FF + 240, 224, 128, 128 + Q4), w))

    for c in in_copies[2:]:
        c.wait()

    def late_prep():
        for a, w_s in enumerate((wr_s, wi_s)):
            last = jnp.concatenate([w_s[DF - 1:DF, :].astype(F32), jnp.zeros((31, S), F32)], axis=0).astype(BF16)
            for j in range(16):
                w32[a, j, 0:112, :] = _pk(w_s[0:DF - 1, 128 * j:128 * j + 128])
                w32[a, j, 112:128, :] = _pk(last[:, 128 * j:128 * j + 128])
        wo = wo_s[...].astype(F32)
        parts = []
        for h in range(H):
            parts += [wo[DH * h:DH * h + DH], jnp.zeros((4, D), F32)]
        wot[...] = _pk(jnp.concatenate(parts, axis=0).astype(BF16).T)

    def tw_pair(k1):
        return tw[8 * k1:8 * k1 + 8, :], tw[128 + 8 * k1:128 + 8 * k1 + 8, :]

    lane = lax.broadcasted_iota(jnp.int32, (8, 128), 1)

    def butterfly(z, h):
        sig = jnp.where((lane & h) == 0, 1.0, -1.0)
        if h == 64:
            return tuple(pltpu.roll(c, 64, 1) + sig * c for c in z)
        low = (lane & h) == 0
        return tuple(jnp.where(low, pltpu.roll(c, 128 - h, 1), pltpu.roll(c, h, 1)) + sig * c for c in z)

    def rot_quarter(z, h, sign):
        m = jnp.logical_and((lane & h) != 0, (lane & (h // 2)) != 0)
        re, im = z
        if sign < 0:
            return jnp.where(m, im, re), jnp.where(m, -re, im)
        return jnp.where(m, -im, re), jnp.where(m, re, im)

    def lane_tw(z, i, sign):
        c, s = tw[256 + 16 * i:264 + 16 * i, :], tw[264 + 16 * i:272 + 16 * i, :]
        re, im = z
        if sign < 0:
            return re * c + im * s, im * c - re * s
        return re * c - im * s, im * c + re * s

    def lane_fft(zs):
        for i, h in enumerate((64, 16, 4)):
            zs = [butterfly(z, h) for z in zs]
            zs = [rot_quarter(z, h, -1) for z in zs]
            zs = [butterfly(z, h // 2) for z in zs]
            zs = [lane_tw(z, i, -1) for z in zs]
        return [butterfly(z, 1) for z in zs]

    def lane_ifft(zs):
        zs = [butterfly(z, 1) for z in zs]
        for i, h in reversed(list(enumerate((64, 16, 4)))):
            zs = [lane_tw(z, i, +1) for z in zs]
            zs = [butterfly(z, h // 2) for z in zs]
            zs = [rot_quarter(z, h, +1) for z in zs]
            zs = [butterfly(z, h) for z in zs]
        return zs

    def filter_rows(a, p_start, shift):
        m10 = (lane & 80) == 64
        m01 = (lane & 80) == 16
        v = []
        for j in range(16):
            w = w32[a, j, pl.ds(p_start, 8, stride=2), :]
            w = pltpu.bitcast((w << shift) & jnp.uint32(0xFFFF0000), F32)
            v.append(jnp.where(m10, pltpu.roll(w, 48, 1), jnp.where(m01, pltpu.roll(w, 80, 1), w)))
        for i in range(4):
            t, d = 1 << i, 8 >> i
            low = (lane & d) == 0
            for j in range(16):
                if j & t == 0:
                    lo, hi = v[j], v[j + t]
                    v[j] = jnp.where(low, lo, pltpu.roll(hi, d, 1))
                    v[j + t] = jnp.where(low, pltpu.roll(lo, 128 - d, 1), hi)
        return [v[int(format(k1, '04b')[::-1], 2)] for k1 in range(16)]

    def spectral_group(gi):
        blk = x1t[pl.ds(pl.multiple_of(gi * 16, 16), 16), :]
        xin = [(blk[0:8, 128 * a:128 * a + 128], blk[8:16, 128 * a:128 * a + 128]) for a in range(16)]
        y = _dft16(xin, -1)
        r = jnp.where(gi < 8, 0, jnp.where(gi < 15, 2, jnp.where(gi < 22, 1, 3)))
        g = gi - jnp.where(gi < 8, 0, jnp.where(gi < 15, 8, jnp.where(gi < 22, 15, 22)))
        p_start = r // 2 + 16 * g
        shift = jnp.asarray(16 - 16 * (r % 2)).astype(U32)
        wr_ = filter_rows(0, p_start, shift)
        wi_ = filter_rows(1, p_start, shift)
        zs = []
        for k1 in range(16):
            re, im = y[k1]
            if k1:
                c, s = tw_pair(k1)
                re, im = re * c + im * s, im * c - re * s
            zs.append((re, im))
        zs = lane_fft(zs)
        zs = [(re * wr_[k1] - im * wi_[k1], re * wi_[k1] + im * wr_[k1]) for k1, (re, im) in enumerate(zs)]
        zs = lane_ifft(zs)
        zin = []
        for k1 in range(16):
            re, im = zs[k1]
            if k1:
                c, s = tw_pair(k1)
                re, im = re * c - im * s, im * c + re * s
            zin.append((re, im))
        z = _dft16(zin, +1)
        top = jnp.concatenate([z[a][0] for a in range(16)], axis=1)
        bot = jnp.concatenate([z[a][1] for a in range(16)], axis=1)
        zt[pl.ds(pl.multiple_of(gi * 8, 8), 8), :] = _pk(jnp.concatenate([top, bot], axis=0).astype(BF16))

    def scores(n):
        h = n // NAQ
        t = h // 4
        i = h % 4
        cols = pl.ds(pl.multiple_of((n % NAQ) * AW, AW), AW)
        q32 = qt[pl.ds(pl.multiple_of(56 * t, 8), 56), cols]
        rr = lax.broadcasted_iota(jnp.int32, (56, AW), 0)
        q32 = jnp.where((rr >= 14 * i) & (rr < 14 * i + 14), q32, jnp.uint32(0))
        qm = _upk(jnp.concatenate([q32, jnp.zeros((8, AW), U32)], axis=0))
        kt = _upk(ks[:, pl.ds(pl.multiple_of(128 * t, 128), 128)])
        return _dot(kt, qm)

    def qk_exp(n, p_ref):
        p_ref[...] = _pk(jnp.exp2(scores(n)).astype(BF16))

    def pv(n, p_ref):
        h = n // NAQ
        rows = pl.ds(pl.multiple_of(16 * h, 16), 16)
        o = _dot(_upk(vt[rows, :]), _upk(p_ref[...]))
        o = o * (1.0 / o[DH:DH + 1, :])
        ot[rows, pl.ds(pl.multiple_of((n % NAQ) * AW, AW), AW)] = _pk(o.astype(BF16))

    @pl.when(safe)
    def _fast():
        late_prep()
        qk_exp(0, p0)

        def body(j, carry):
            qk_exp(2 * j + 1, p1)
            pv(2 * j, p0)
            qk_exp(2 * j + 2, p0)
            pv(2 * j + 1, p1)
            for m in range(GPI):
                spectral_group(jnp.minimum(GPI * j + m, NG - 1))
            return carry

        lax.fori_loop(0, NIT, body, 0)
        qk_exp(NBLK - 1, p1)
        pv(NBLK - 2, p0)
        pv(NBLK - 1, p1)
        for gi in range(NIT * GPI, NG):
            spectral_group(gi)

    @pl.when(jnp.logical_not(safe))
    def _slow():
        late_prep()

        def body(n, carry):
            sbuf[...] = scores(n)
            m = jnp.max(jnp.max(sbuf[...].reshape(S // 8, 8, AW), axis=0), axis=0, keepdims=True)
            p0[...] = _pk(jnp.exp2(sbuf[...] - m).astype(BF16))
            pv(n, p0)
            return carry

        lax.fori_loop(0, NBLK, body, 0)

        def fbody(gi, carry):
            spectral_group(gi)
            return carry

        lax.fori_loop(0, NG, fbody, 0)

    def out_copy(b):
        c = pl.ds(pl.multiple_of(b * QB, QB), QB)
        return pltpu.make_async_copy(outb.at[:, c], out_hbm.at[:, c], sem_out.at[b])

    def final_block(b, carry):
        cols = pl.ds(b * QB, QB)
        at = _dot(_upk(wot[...]), _upk(ot[:, cols]))
        t0 = _dot(cbt(_O_G0, Q4, 0, 128), _upk(zt[0:64, cols]))
        t2 = _dot(cbt(_O_G2, Q4, 0, Q4), _upk(zt[64:120, cols]))
        ab = _dot(cbt(_O_GAB, 2 * Q4, 0, 2 * Q4), _upk(zt[120:232, cols]))
        e, o = t0 + t2, t0 - t2
        yt = jnp.concatenate([e + ab[0:Q4], o + ab[Q4:], e - ab[0:Q4], o - ab[Q4:]], axis=0)
        g = jax.nn.sigmoid(gt[0:1, cols])
        outb[:, cols] = (g * at + (1.0 - g) * yt).astype(BF16)
        out_copy(b).start()
        return carry

    for b in range(NQB):
        final_block(b, 0)
    for b in range(NQB):
        out_copy(b).wait()


@jax.jit
def pallas_gated_mix__softmax_full_mha__spectral_gfnet__prompt_kernel(
    A_x: jax.Array,
    A_wqkv: jax.Array,
    A_wo: jax.Array,
    B_x: jax.Array,
    B_w_r: jax.Array,
    B_w_i: jax.Array,
    gate_w: jax.Array,
):
    del B_x
    cb_np, tw_np = _tables()
    any_spec = pl.BlockSpec(memory_space=pltpu.HBM)
    scratch = [
        pltpu.VMEM((D, S), BF16),
        pltpu.VMEM((D, 3 * D), BF16),
        pltpu.VMEM((D, D), BF16),
        pltpu.VMEM((DF, S), BF16),
        pltpu.VMEM((DF, S), BF16),
        pltpu.VMEM((D,), BF16),
        pltpu.VMEM(cb_np.shape, U32),
        pltpu.VMEM(tw_np.shape, F32),
        pltpu.VMEM((3 * D // 2 + 8, D), U32),
        pltpu.VMEM((D // 2, 512), U32),
        pltpu.VMEM((S // 2, 512), U32),
        pltpu.VMEM((D // 2, S), U32),
        pltpu.VMEM((256, S), U32),
        pltpu.VMEM((256, S), U32),
        pltpu.VMEM((8, S), F32),
        pltpu.VMEM((S // 2, AW), U32),
        pltpu.VMEM((S // 2, AW), U32),
        pltpu.VMEM((NROW, S), F32),
        pltpu.VMEM((2, 16, 128, 128), U32),
        pltpu.VMEM((NROW // 2, S), U32),
        pltpu.VMEM((D, S), BF16),
        pltpu.VMEM((S, AW), F32),
        pltpu.SemaphoreType.DMA((NQB,)),
        pltpu.SemaphoreType.DMA((4,)),
        pltpu.SemaphoreType.DMA((6,)),
        pltpu.SemaphoreType.DMA((NQB,)),
    ]
    out = pl.pallas_call(
        _kernel,
        out_shape=jax.ShapeDtypeStruct((D, S), BF16),
        in_specs=[any_spec] * 8,
        out_specs=any_spec,
        scratch_shapes=scratch,
        compiler_params=pltpu.CompilerParams(vmem_limit_bytes=100 * 1024 * 1024),
    )(A_x.reshape(S, D).T, A_wqkv, A_wo, B_w_r.T, B_w_i.T, gate_w, jnp.asarray(cb_np), jnp.asarray(tw_np))
    return out.T.reshape(1, S, D)
```

```python
import functools

import numpy as np
import jax
import jax.numpy as jnp
from jax import lax
import jax.experimental.pallas as pl
import jax.experimental.pallas.tpu as pltpu

F32 = jnp.float32
BF16 = jnp.bfloat16
U32 = jnp.uint32

S, D, H, DH = 2048, 448, 16, 28
DF = D // 2 + 1
Q4 = D // 4
QB = 512
NQB = S // QB
AW = 1024
NAQ = S // AW
NBLK = H * NAQ
NIT = NBLK // 2 - 1
GPI = 2

E8 = D // 8
_TILES = ((0, 4), (2, 6), (1, 7), (3, 5))


def _tile_freqs(r, rc):
    a = list(range(r, DF, 8))
    b = list(range(rc, DF, 8))
    out = a[0:28] + b[24:28] + b[0:24]
    if len(a) > 28:
        out += a[28:] + [-1] * (8 - len(a[28:]))
    return out


_FREQS = [_tile_freqs(*t) for t in _TILES]
_ROW0 = [0]
for _f in _FREQS:
    _ROW0.append(_ROW0[-1] + 2 * len(_f))
NROW = _ROW0[-1]
NG = NROW // 16


def _pack_rows_np(a):
    u = np.ascontiguousarray(a, dtype=np.float32).view(np.uint32)
    b = ((u + 0x7FFF + ((u >> 16) & 1)) >> 16).astype(np.uint32)
    return b[0::2] | (b[1::2] << 16)


@functools.lru_cache(maxsize=1)
def _tables():
    dp = np.arange(E8)
    ff = np.zeros((NROW, 128), np.float64)
    gg = np.zeros((4 * Q4, 128), np.float64)
    norm = 1.0 / (S * D)
    for t, fl in enumerate(_FREQS):
        for pos, f in enumerate(fl):
            if f < 0:
                continue
            th = 2 * np.pi * f * dp / D
            c, s = np.cos(th), np.sin(th)
            cf = (1.0 if f in (0, D // 2) else 2.0) * norm
            first = f % 8 == _TILES[t][0]
            sg = 1.0 if first else -1.0
            for im in (0, 1):
                col = 16 * (pos // 8) + 8 * im + pos % 8
                row = _ROW0[t] + col
                re_part = (-s if im else c) * cf
                im_part = (c if im else s) * cf
                if t == 0:
                    half = 0 if first else E8
                    ff[row, half:half + E8] = -s if im else c
                    gg[half:half + E8, col] = re_part
                else:
                    ff[row, :E8] = -s if im else c
                    ff[row, E8:2 * E8] = sg * c if im else sg * s
                    gg[Q4 * t:Q4 * t + E8, col] = re_part
                    gg[Q4 * t + E8:Q4 * t + 2 * E8, col] = sg * im_part
    b = np.arange(128)
    tw = 2 * np.pi * np.outer(np.arange(16), b) / S
    rows_tw = [np.repeat(np.cos(tw), 8, axis=0), np.repeat(np.sin(tw), 8, axis=0)]
    for h in (64, 16, 4):
        ang = 2 * np.pi * (b % (h // 2)) * (((b & h) != 0) * 1 + ((b & (h // 2)) != 0) * 2) / (2 * h)
        rows_tw += [np.repeat(np.cos(ang)[None], 8, axis=0), np.repeat(np.sin(ang)[None], 8, axis=0)]
    twid = np.concatenate(rows_tw, 0)
    return _pack_rows_np(ff), _pack_rows_np(gg), twid.astype(np.float32)


def _pk(x):
    return pltpu.bitcast(x, U32)


def _upk(x):
    return pltpu.bitcast(x, BF16)


def _dot(a, b):
    return jnp.dot(a, b, preferred_element_type=F32)


def _dot_nt(a, b):
    return lax.dot_general(a, b, (((1,), (1,)), ((), ())), preferred_element_type=F32)


def _cmul_const(z, ang):
    re, im = z
    k = int(round(ang / (2 * np.pi / 16))) % 16
    if k == 0:
        return z
    if k == 4:
        return (-im, re)
    if k == 8:
        return (-re, -im)
    if k == 12:
        return (im, -re)
    c, s = float(np.cos(ang)), float(np.sin(ang))
    if k % 4 == 2:
        a = abs(c)
        p, m = (re + im) * a, (re - im) * a
        if k == 2:
            return (m, p)
        if k == 6:
            return (-p, m)
        if k == 10:
            return (-m, -p)
        return (p, -m)
    return (re * c - im * s, re * s + im * c)


def _dft4(x, sign):
    (r0, i0), (r1, i1), (r2, i2), (r3, i3) = x
    ar, ai = r0 + r2, i0 + i2
    br, bi = r0 - r2, i0 - i2
    cr, ci = r1 + r3, i1 + i3
    dr, di = r1 - r3, i1 - i3
    y0 = (ar + cr, ai + ci)
    y2 = (ar - cr, ai - ci)
    ym = (br + di, bi - dr)
    yp = (br - di, bi + dr)
    return [y0, ym, y2, yp] if sign < 0 else [y0, yp, y2, ym]


def _dft16(x, sign):
    a = [_dft4([x[4 * n1 + n0] for n1 in range(4)], sign) for n0 in range(4)]
    out = [None] * 16
    for k0 in range(4):
        col = [_cmul_const(a[n0][k0], sign * 2 * np.pi * n0 * k0 / 16) for n0 in range(4)]
        y = _dft4(col, sign)
        for k1 in range(4):
            out[k0 + 4 * k1] = y[k1]
    return out


_RS2 = float(np.sqrt(0.5))

_SAFE_SCORE = 60.0
_V_HI = 2.0 ** 50
_V_LO = 2.0 ** -40


def _kernel(xt_hbm, wqkv_hbm, wo_hbm, wr_hbm, wi_hbm, gate_hbm, ff_hbm, gg_hbm, tw_hbm, out_hbm,
            xs, wq_s, wo_s, wr_s, wi_s, gate_s, ff, gg, tw,
            lhs_all, wot, ks, qt, vt, ot, gt,
            p0, p1, x1t, w32, zt, outb, sbuf,
            sem_x, sem_w, sem_in, sem_out):
    def x_copy(b):
        c = pl.ds(pl.multiple_of(b * QB, QB), QB)
        return pltpu.make_async_copy(xt_hbm.at[:, c], xs.at[:, c], sem_x.at[b])

    w_chunks = [(128 * c, min(128, 3 * D - 128 * c)) for c in range(11)]
    w_copies = [pltpu.make_async_copy(wqkv_hbm.at[:, pl.ds(o, n)], wq_s.at[:, pl.ds(o, n)], sem_w.at[i])
                for i, (o, n) in enumerate(w_chunks)]
    in_copies = [
        pltpu.make_async_copy(src, dst, sem_in.at[i])
        for i, (src, dst) in enumerate([(gate_hbm, gate_s), (ff_hbm, ff), (tw_hbm, tw),
                                        (wo_hbm, wo_s), (wr_hbm, wr_s), (wi_hbm, wi_s), (gg_hbm, gg)])]
    x_copy(0).start()
    in_copies[1].start()
    for c in w_copies[0:4]:
        c.start()


    def prep_w(lo, hi, wait=True):
        for i in range(lo, hi):
            if wait:
                w_copies[i].wait()
        for i in range(lo, hi):
            o, n = w_chunks[i]
            lhs_all[o // 2:(o + n) // 2, :] = _pk(wq_s[:, o:o + n].T)

    qscale = float(DH ** -0.5 * np.log2(np.e))

    def lane_tile_max(a):
        parts = [a[:, 128 * j:128 * j + 128] for j in range(a.shape[1] // 128)]
        while len(parts) > 1:
            parts = [jnp.maximum(parts[i], parts[i + 1]) if i + 1 < len(parts) else parts[i]
                     for i in range(0, len(parts), 2)]
        return parts[0]

    def proj_q(c0, n, qv):
        q = (qv * qscale).astype(BF16)
        qt[:, c0:c0 + n] = _pk(q)
        return lane_tile_max(jnp.abs(q.astype(F32)))

    def proj_k(c0, n, kv):
        k = kv.astype(BF16)
        for t in range(4):
            kg = jnp.concatenate([k[Q4 * t:Q4 * t + Q4], jnp.zeros((16, n), BF16)], axis=0)
            ks[c0 // 2:(c0 + n) // 2, 128 * t:128 * t + 128] = _pk(kg.T)
        return lane_tile_max(jnp.abs(k.astype(F32)))

    def proj_v(c0, n, v, glogit):
        tail = (lax.broadcasted_iota(jnp.int32, (4, n), 0) == 0).astype(F32)
        parts = []
        for h in range(H):
            parts += [v[DH * h:DH * h + DH], tail]
        vt[:, c0:c0 + n] = _pk(jnp.concatenate(parts, axis=0).astype(BF16))
        gt[:, c0:c0 + n] = jnp.broadcast_to(glogit, (8, n))
        return lane_tile_max(jnp.max(jnp.abs(v).reshape(D // 8, 8, n), axis=0))

    def proj_block(c0, n):
        qkv = _dot(_upk(lhs_all[...]), xs[:, c0:c0 + n])
        return (proj_q(c0, n, qkv[0:D]), proj_k(c0, n, qkv[D:2 * D]),
                proj_v(c0, n, qkv[2 * D:3 * D], qkv[3 * D:3 * D + 1]))

    def dft_d_block(c0, n):
        cols = slice(c0, c0 + n)
        xf = xs[:, cols].astype(F32)
        xj = [xf[E8 * j:E8 * j + E8] for j in range(8)]
        a = [xj[j] + xj[j + 4] for j in range(4)]
        b = [xj[j] - xj[j + 4] for j in range(4)]
        ae, ao = a[0] + a[2], a[1] + a[3]
        p, q = (b[1] - b[3]) * _RS2, (b[1] + b[3]) * _RS2
        ops = [(ae + ao, ae - ao), (a[0] - a[2], a[3] - a[1]), (b[0] + p, -(b[2] + q)), (b[0] - p, b[2] - q)]
        for t in range(4):
            y = jnp.concatenate(ops[t], axis=0).astype(BF16)
            lhs = _upk(ff[_ROW0[t] // 2:_ROW0[t + 1] // 2, :])[:, 0:Q4]
            x1t[_ROW0[t]:_ROW0[t + 1], cols] = _dot(lhs, y)

    x_copy(0).wait()
    in_copies[1].wait()
    for c in w_copies[0:4]:
        c.wait()
    for c in w_copies[4:7]:
        c.start()
    prep_w(0, 4, wait=False)
    dft_d_block(0, QB)
    xb0 = xs[:, 0:QB]
    for c in w_copies[4:6]:
        c.wait()
    for c in w_copies[7:]:
        c.start()
    in_copies[0].start()
    w_copies[6].wait()
    prep_w(4, 7, wait=False)
    amax0 = proj_q(0, QB, _dot(_upk(lhs_all[0:D // 2, :]), xb0))
    for b in range(1, NQB):
        x_copy(b).start()
    for c in w_copies[7:]:
        c.wait()
    in_copies[0].wait()
    prep_w(7, 11, wait=False)
    gate16 = jnp.concatenate([gate_s[...].reshape(1, D).astype(F32), jnp.zeros((15, D), F32)], axis=0)
    lhs_all[3 * D // 2:3 * D // 2 + 8, :] = _pk(gate16.astype(BF16))
    kmax0 = proj_k(0, QB, _dot(_upk(lhs_all[D // 2:D, :]), xb0))
    vg = _dot(_upk(lhs_all[D:3 * D // 2 + 8, :]), xb0)
    st = [(amax0, kmax0, proj_v(0, QB, vg[0:D], vg[D:D + 1]))]
    for c in in_copies[2:]:
        c.start()
    for b in range(1, NQB):
        x_copy(b).wait()
    st.append(proj_block(QB, QB))
    st.append(proj_block(2 * QB, QB))
    dft_d_block(QB, QB)
    st.append(proj_block(3 * QB, QB))
    dft_d_block(2 * QB, QB)
    dft_d_block(3 * QB, QB)
    amax, kmax, vmax = [jnp.maximum(jnp.maximum(a, b), jnp.maximum(c, d)) for a, b, c, d in zip(*st)]

    kcol = jnp.max(kmax, axis=1, keepdims=True)
    prod = (amax * kcol).astype(BF16)
    hh = lax.broadcasted_iota(jnp.int32, (H, D), 0)
    jj = lax.broadcasted_iota(jnp.int32, (H, D), 1)
    ind = jnp.where((jj >= DH * hh) & (jj < DH * hh + DH), 1.0, 0.0).astype(BF16)
    bound = jnp.max(_dot(ind, prod)) * 1.03
    vmax = jnp.max(vmax)
    safe = jnp.logical_and(bound <= _SAFE_SCORE, jnp.logical_and(vmax <= _V_HI, vmax >= _V_LO))

    for c in in_copies[2:]:
        c.wait()

    def late_prep():
        for a, w_s in enumerate((wr_s, wi_s)):
            last = jnp.concatenate([w_s[DF - 1:DF, :].astype(F32), jnp.zeros((63, S), F32)], axis=0).astype(BF16)
            for j in range(16):
                w32[a, j, 0:112, :] = _pk(w_s[0:DF - 1, 128 * j:128 * j + 128])
                w32[a, j, 112:144, :] = _pk(last[:, 128 * j:128 * j + 128])
        wo = wo_s[...].astype(F32)
        parts = []
        for h in range(H):
            parts += [wo[DH * h:DH * h + DH], jnp.zeros((4, D), F32)]
        wot[...] = _pk(jnp.concatenate(parts, axis=0).astype(BF16).T)

    def tw_pair(k1):
        return tw[8 * k1:8 * k1 + 8, :], tw[128 + 8 * k1:128 + 8 * k1 + 8, :]

    lane = lax.broadcasted_iota(jnp.int32, (8, 128), 1)

    def butterfly(z, h):
        sig = jnp.where((lane & h) == 0, 1.0, -1.0)
        if h == 64:
            return tuple(pltpu.roll(c, 64, 1) + sig * c for c in z)
        low = (lane & h) == 0
        return tuple(jnp.where(low, pltpu.roll(c, 128 - h, 1), pltpu.roll(c, h, 1)) + sig * c for c in z)

    def rot_quarter(z, h, sign):
        m = jnp.logical_and((lane & h) != 0, (lane & (h // 2)) != 0)
        re, im = z
        if sign < 0:
            return jnp.where(m, im, re), jnp.where(m, -re, im)
        return jnp.where(m, -im, re), jnp.where(m, re, im)

    def lane_tw(z, i, sign):
        c, s = tw[256 + 16 * i:264 + 16 * i, :], tw[264 + 16 * i:272 + 16 * i, :]
        re, im = z
        if sign < 0:
            return re * c + im * s, im * c - re * s
        return re * c - im * s, im * c + re * s

    def lane_fft(zs):
        for i, h in enumerate((64, 16, 4)):
            zs = [butterfly(z, h) for z in zs]
            zs = [rot_quarter(z, h, -1) for z in zs]
            zs = [butterfly(z, h // 2) for z in zs]
            zs = [lane_tw(z, i, -1) for z in zs]
        return [butterfly(z, 1) for z in zs]

    def lane_ifft(zs):
        zs = [butterfly(z, 1) for z in zs]
        for i, h in reversed(list(enumerate((64, 16, 4)))):
            zs = [lane_tw(z, i, +1) for z in zs]
            zs = [butterfly(z, h // 2) for z in zs]
            zs = [rot_quarter(z, h, +1) for z in zs]
            zs = [butterfly(z, h) for z in zs]
        return zs

    def filter_rows(a, pa, pb, shift):
        m10 = (lane & 80) == 64
        m01 = (lane & 80) == 16
        top4 = lax.broadcasted_iota(jnp.int32, (8, 128), 0) < 4
        v = []
        for j in range(16):
            w = jnp.where(top4, w32[a, j, pl.ds(pa, 8, stride=4), :], w32[a, j, pl.ds(pb, 8, stride=4), :])
            w = pltpu.bitcast((w << shift) & jnp.uint32(0xFFFF0000), F32)
            v.append(jnp.where(m10, pltpu.roll(w, 48, 1), jnp.where(m01, pltpu.roll(w, 80, 1), w)))
        for i in range(4):
            t, d = 1 << i, 8 >> i
            low = (lane & d) == 0
            for j in range(16):
                if j & t == 0:
                    lo, hi = v[j], v[j + t]
                    v[j] = jnp.where(low, lo, pltpu.roll(hi, d, 1))
                    v[j + t] = jnp.where(low, pltpu.roll(lo, 128 - d, 1), hi)
        return [v[int(format(k1, '04b')[::-1], 2)] for k1 in range(16)]

    def spectral_group(gi):
        blk = x1t[pl.ds(pl.multiple_of(gi * 16, 16), 16), :]
        xin = [(blk[0:8, 128 * a:128 * a + 128], blk[8:16, 128 * a:128 * a + 128]) for a in range(16)]
        y = _dft16(xin, -1)
        t1, t2, t3 = gi >= 8, gi >= 15, gi >= 22
        r = jnp.where(t3, 3, jnp.where(t2, 1, jnp.where(t1, 2, 0)))
        rc = jnp.where(t3, 5, jnp.where(t2, 7, jnp.where(t1, 6, 4)))
        g = gi - jnp.where(t3, 22, jnp.where(t2, 15, jnp.where(t1, 8, 0)))
        fa = jnp.where(g < 4, r + 64 * g, jnp.where(g < 7, rc + 64 * (g - 4), D // 2))
        fb = jnp.where(g == 3, rc + 192, fa + 32)
        pa, pb = fa // 2, fb // 2 - 16
        shift = jnp.asarray(16 - 16 * (r % 2)).astype(U32)
        wr_ = filter_rows(0, pa, pb, shift)
        wi_ = filter_rows(1, pa, pb, shift)
        zs = []
        for k1 in range(16):
            re, im = y[k1]
            if k1:
                c, s = tw_pair(k1)
                re, im = re * c + im * s, im * c - re * s
            zs.append((re, im))
        zs = lane_fft(zs)
        zs = [(re * wr_[k1] - im * wi_[k1], re * wi_[k1] + im * wr_[k1]) for k1, (re, im) in enumerate(zs)]
        zs = lane_ifft(zs)
        zin = []
        for k1 in range(16):
            re, im = zs[k1]
            if k1:
                c, s = tw_pair(k1)
                re, im = re * c - im * s, im * c + re * s
            zin.append((re, im))
        z = _dft16(zin, +1)
        top = jnp.concatenate([z[a][0] for a in range(16)], axis=1)
        bot = jnp.concatenate([z[a][1] for a in range(16)], axis=1)
        zt[pl.ds(pl.multiple_of(gi * 8, 8), 8), :] = _pk(jnp.concatenate([top, bot], axis=0).astype(BF16))

    def scores(n):
        h = n // NAQ
        t = h // 4
        i = h % 4
        cols = pl.ds(pl.multiple_of((n % NAQ) * AW, AW), AW)
        q32 = qt[pl.ds(pl.multiple_of(56 * t, 8), 56), cols]
        rr = lax.broadcasted_iota(jnp.int32, (56, AW), 0)
        q32 = jnp.where((rr >= 14 * i) & (rr < 14 * i + 14), q32, jnp.uint32(0))
        qm = _upk(jnp.concatenate([q32, jnp.zeros((8, AW), U32)], axis=0))
        kt = _upk(ks[:, pl.ds(pl.multiple_of(128 * t, 128), 128)])
        return _dot(kt, qm)

    def qk_exp(n, p_ref):
        p_ref[...] = _pk(jnp.exp2(scores(n)).astype(BF16))

    def pv(n, p_ref):
        h = n // NAQ
        rows = pl.ds(pl.multiple_of(16 * h, 16), 16)
        o = _dot(_upk(vt[rows, :]), _upk(p_ref[...]))
        o = o * (1.0 / o[DH:DH + 1, :])
        ot[rows, pl.ds(pl.multiple_of((n % NAQ) * AW, AW), AW)] = _pk(o.astype(BF16))

    @pl.when(safe)
    def _fast():
        late_prep()
        qk_exp(0, p0)

        def body(j, carry):
            qk_exp(2 * j + 1, p1)
            pv(2 * j, p0)
            qk_exp(2 * j + 2, p0)
            pv(2 * j + 1, p1)
            for m in range(GPI):
                spectral_group(jnp.minimum(GPI * j + m, NG - 1))
            return carry

        lax.fori_loop(0, NIT, body, 0)
        qk_exp(NBLK - 1, p1)
        pv(NBLK - 2, p0)
        pv(NBLK - 1, p1)
        for gi in range(NIT * GPI, NG):
            spectral_group(gi)

    @pl.when(jnp.logical_not(safe))
    def _slow():
        late_prep()

        def body(n, carry):
            sbuf[...] = scores(n)
            m = jnp.max(jnp.max(sbuf[...].reshape(S // 8, 8, AW), axis=0), axis=0, keepdims=True)
            p0[...] = _pk(jnp.exp2(sbuf[...] - m).astype(BF16))
            pv(n, p0)
            return carry

        lax.fori_loop(0, NBLK, body, 0)

        def fbody(gi, carry):
            spectral_group(gi)
            return carry

        lax.fori_loop(0, NG, fbody, 0)

    out_blocks = [(0, 512), (512, 512), (1024, 512), (1536, 384), (1920, 128)]

    def out_copy(b):
        c = pl.ds(*out_blocks[b])
        return pltpu.make_async_copy(outb.at[:, c], out_hbm.at[:, c], sem_out.at[b])

    for b, (c0, n) in enumerate(out_blocks):
        cols = slice(c0, c0 + n)
        tt = []
        for t in range(4):
            k = _ROW0[t + 1] - _ROW0[t]
            r_ = _dot(_upk(gg[Q4 * t // 2:Q4 * (t + 1) // 2, :])[:, 0:k], _upk(zt[_ROW0[t] // 2:_ROW0[t + 1] // 2, cols]))
            tt.append((r_[0:E8], r_[E8:2 * E8]))
        (t0, t4), (a2, b2), (a1, b1), (a3, b3) = tt
        ee, eo = t0 + t4, t0 - t4
        m1, p1_ = (a1 - b1) * _RS2, (a1 + b1) * _RS2
        m3, p3 = (a3 - b3) * _RS2, (a3 + b3) * _RS2
        u0, u2, u1, u3 = ee + a2, ee - a2, eo - b2, eo + b2
        w0, w2, w1, w3 = a1 + a3, b3 - b1, m1 - p3, m3 - p1_
        yt = jnp.concatenate([u0 + w0, u1 + w1, u2 + w2, u3 + w3, u0 - w0, u1 - w1, u2 - w2, u3 - w3], axis=0)
        g = jax.nn.sigmoid(gt[0:1, cols])
        yt = (1.0 - g) * yt
        at = _dot(_upk(wot[...]), _upk(ot[:, cols]))
        outb[:, cols] = (g * at + yt).astype(BF16)
        out_copy(b).start()
    for b in range(len(out_blocks)):
        out_copy(b).wait()


@jax.jit
def pallas_gated_mix__softmax_full_mha__spectral_gfnet__prompt_kernel(
    A_x: jax.Array,
    A_wqkv: jax.Array,
    A_wo: jax.Array,
    B_x: jax.Array,
    B_w_r: jax.Array,
    B_w_i: jax.Array,
    gate_w: jax.Array,
):
    del B_x
    ff_np, gg_np, tw_np = _tables()
    any_spec = pl.BlockSpec(memory_space=pltpu.HBM)
    scratch = [
        pltpu.VMEM((D, S), BF16),
        pltpu.VMEM((D, 3 * D), BF16),
        pltpu.VMEM((D, D), BF16),
        pltpu.VMEM((DF, S), BF16),
        pltpu.VMEM((DF, S), BF16),
        pltpu.VMEM((D,), BF16),
        pltpu.VMEM(ff_np.shape, U32),
        pltpu.VMEM(gg_np.shape, U32),
        pltpu.VMEM(tw_np.shape, F32),
        pltpu.VMEM((3 * D // 2 + 8, D), U32),
        pltpu.VMEM((D // 2, 512), U32),
        pltpu.VMEM((S // 2, 512), U32),
        pltpu.VMEM((D // 2, S), U32),
        pltpu.VMEM((256, S), U32),
        pltpu.VMEM((256, S), U32),
        pltpu.VMEM((8, S), F32),
        pltpu.VMEM((S // 2, AW), U32),
        pltpu.VMEM((S // 2, AW), U32),
        pltpu.VMEM((NROW, S), F32),
        pltpu.VMEM((2, 16, 144, 128), U32),
        pltpu.VMEM((NROW // 2, S), U32),
        pltpu.VMEM((D, S), BF16),
        pltpu.VMEM((S, AW), F32),
        pltpu.SemaphoreType.DMA((NQB,)),
        pltpu.SemaphoreType.DMA((11,)),
        pltpu.SemaphoreType.DMA((7,)),
        pltpu.SemaphoreType.DMA((5,)),
    ]
    out = pl.pallas_call(
        _kernel,
        out_shape=jax.ShapeDtypeStruct((D, S), BF16),
        in_specs=[any_spec] * 9,
        out_specs=any_spec,
        scratch_shapes=scratch,
        compiler_params=pltpu.CompilerParams(vmem_limit_bytes=100 * 1024 * 1024),
    )(A_x.reshape(S, D).T, A_wqkv, A_wo, B_w_r.T, B_w_i.T, gate_w,
      jnp.asarray(ff_np), jnp.asarray(gg_np), jnp.asarray(tw_np))
    return out.T.reshape(1, S, D)
```

```python
import functools

import numpy as np
import jax
import jax.numpy as jnp
from jax import lax
import jax.experimental.pallas as pl
import jax.experimental.pallas.tpu as pltpu

F32 = jnp.float32
BF16 = jnp.bfloat16
U32 = jnp.uint32

S, D, H, DH = 2048, 448, 16, 28
DF = D // 2 + 1
Q4 = D // 4
QB = 512
NQB = S // QB
AW = 1024
NAQ = S // AW
NBLK = H * NAQ
NIT = NBLK // 2 - 1
GPI = 2

E8 = D // 8
_TILES = ((0, 4), (2, 6), (1, 7), (3, 5))


def _tile_freqs(r, rc):
    a = list(range(r, DF, 8))
    b = list(range(rc, DF, 8))
    out = a[0:28] + b[24:28] + b[0:24]
    if len(a) > 28:
        out += a[28:] + [-1] * (8 - len(a[28:]))
    return out


_FREQS = [_tile_freqs(*t) for t in _TILES]
_ROW0 = [0]
for _f in _FREQS:
    _ROW0.append(_ROW0[-1] + 2 * len(_f))
NROW = _ROW0[-1]
NG = NROW // 16


def _pack_rows_np(a):
    u = np.ascontiguousarray(a, dtype=np.float32).view(np.uint32)
    b = ((u + 0x7FFF + ((u >> 16) & 1)) >> 16).astype(np.uint32)
    return b[0::2] | (b[1::2] << 16)


@functools.lru_cache(maxsize=1)
def _tables():
    dp = np.arange(E8)
    ff = np.zeros((NROW, 128), np.float64)
    gg = np.zeros((4 * Q4, 128), np.float64)
    norm = 1.0 / (S * D)
    for t, fl in enumerate(_FREQS):
        for pos, f in enumerate(fl):
            if f < 0:
                continue
            th = 2 * np.pi * f * dp / D
            c, s = np.cos(th), np.sin(th)
            cf = (1.0 if f in (0, D // 2) else 2.0) * norm
            first = f % 8 == _TILES[t][0]
            sg = 1.0 if first else -1.0
            for im in (0, 1):
                col = 16 * (pos // 8) + 8 * im + pos % 8
                row = _ROW0[t] + col
                re_part = (-s if im else c) * cf
                im_part = (c if im else s) * cf
                if t == 0:
                    half = 0 if first else E8
                    ff[row, half:half + E8] = -s if im else c
                    gg[half:half + E8, col] = re_part
                else:
                    ff[row, :E8] = -s if im else c
                    ff[row, E8:2 * E8] = sg * c if im else sg * s
                    gg[Q4 * t:Q4 * t + E8, col] = re_part
                    gg[Q4 * t + E8:Q4 * t + 2 * E8, col] = sg * im_part
    b = np.arange(128)
    tw = 2 * np.pi * np.outer(np.arange(16), b) / S
    rows_tw = [np.repeat(np.cos(tw), 8, axis=0), np.repeat(np.sin(tw), 8, axis=0)]
    for h in (64, 16, 4):
        ang = 2 * np.pi * (b % (h // 2)) * (((b & h) != 0) * 1 + ((b & (h // 2)) != 0) * 2) / (2 * h)
        rows_tw += [np.repeat(np.cos(ang)[None], 8, axis=0), np.repeat(np.sin(ang)[None], 8, axis=0)]
    twid = np.concatenate(rows_tw, 0)
    return _pack_rows_np(ff), _pack_rows_np(gg), twid.astype(np.float32)


def _pk(x):
    return pltpu.bitcast(x, U32)


def _upk(x):
    return pltpu.bitcast(x, BF16)


def _dot(a, b):
    return jnp.dot(a, b, preferred_element_type=F32)


def _cmul_const(z, ang):
    re, im = z
    k = int(round(ang / (2 * np.pi / 16))) % 16
    if k == 0:
        return z
    if k == 4:
        return (-im, re)
    if k == 8:
        return (-re, -im)
    if k == 12:
        return (im, -re)
    c, s = float(np.cos(ang)), float(np.sin(ang))
    if k % 4 == 2:
        a = abs(c)
        p, m = (re + im) * a, (re - im) * a
        if k == 2:
            return (m, p)
        if k == 6:
            return (-p, m)
        if k == 10:
            return (-m, -p)
        return (p, -m)
    return (re * c - im * s, re * s + im * c)


def _dft4(x, sign):
    (r0, i0), (r1, i1), (r2, i2), (r3, i3) = x
    ar, ai = r0 + r2, i0 + i2
    br, bi = r0 - r2, i0 - i2
    cr, ci = r1 + r3, i1 + i3
    dr, di = r1 - r3, i1 - i3
    y0 = (ar + cr, ai + ci)
    y2 = (ar - cr, ai - ci)
    ym = (br + di, bi - dr)
    yp = (br - di, bi + dr)
    return [y0, ym, y2, yp] if sign < 0 else [y0, yp, y2, ym]


def _dft16(x, sign):
    a = [_dft4([x[4 * n1 + n0] for n1 in range(4)], sign) for n0 in range(4)]
    out = [None] * 16
    for k0 in range(4):
        col = [_cmul_const(a[n0][k0], sign * 2 * np.pi * n0 * k0 / 16) for n0 in range(4)]
        y = _dft4(col, sign)
        for k1 in range(4):
            out[k0 + 4 * k1] = y[k1]
    return out


_RS2 = float(np.sqrt(0.5))

_SAFE_SCORE = 60.0
_V_HI = 2.0 ** 50
_V_LO = 2.0 ** -40


def _kernel(xt_hbm, wqkv_hbm, wo_hbm, wr_hbm, wi_hbm, gate_hbm, ff_hbm, gg_hbm, tw_hbm, out_hbm,
            xs, wq_s, wo_s, wr_s, wi_s, gate_s, ff, gg, tw,
            lhs_all, wot, ks, qt, vt, ot, gt,
            p0, p1, x1t, w32, zt, outb, sbuf,
            sem_x, sem_w, sem_in, sem_out):
    def x_copy(b):
        c = pl.ds(pl.multiple_of(b * QB, QB), QB)
        return pltpu.make_async_copy(xt_hbm.at[:, c], xs.at[:, c], sem_x.at[b])

    w_chunks = [(128 * c, min(128, 3 * D - 128 * c)) for c in range(11)]
    w_copies = [pltpu.make_async_copy(wqkv_hbm.at[:, pl.ds(o, n)], wq_s.at[:, pl.ds(o, n)], sem_w.at[i])
                for i, (o, n) in enumerate(w_chunks)]
    in_copies = [
        pltpu.make_async_copy(src, dst, sem_in.at[i])
        for i, (src, dst) in enumerate([(gate_hbm, gate_s), (ff_hbm, ff), (tw_hbm, tw),
                                        (wo_hbm, wo_s), (wr_hbm, wr_s), (wi_hbm, wi_s), (gg_hbm, gg)])]
    x_copy(0).start()
    in_copies[1].start()
    for c in w_copies[0:4]:
        c.start()

    def prep_w(lo, hi, wait=True):
        for i in range(lo, hi):
            if wait:
                w_copies[i].wait()
        for i in range(lo, hi):
            o, n = w_chunks[i]
            lhs_all[o // 2:(o + n) // 2, :] = _pk(wq_s[:, o:o + n].T)

    qscale = float(DH ** -0.5 * np.log2(np.e))

    def lane_tile_max(a):
        parts = [a[:, 128 * j:128 * j + 128] for j in range(a.shape[1] // 128)]
        while len(parts) > 1:
            parts = [jnp.maximum(parts[i], parts[i + 1]) if i + 1 < len(parts) else parts[i]
                     for i in range(0, len(parts), 2)]
        return parts[0]

    def proj_q(c0, n, qv):
        q = qv * qscale
        qt[:, c0:c0 + n] = _pk(q.astype(BF16))
        return lane_tile_max(jnp.abs(q))

    def proj_k(c0, n, kv):
        k = kv.astype(BF16)
        for t in range(4):
            kg = jnp.concatenate([k[Q4 * t:Q4 * t + Q4], jnp.zeros((16, n), BF16)], axis=0)
            ks[c0 // 2:(c0 + n) // 2, 128 * t:128 * t + 128] = _pk(kg.T)
        return lane_tile_max(jnp.abs(kv))

    def proj_v(c0, n, v, glogit):
        tail = (lax.broadcasted_iota(jnp.int32, (4, n), 0) == 0).astype(F32)
        parts = []
        for h in range(H):
            parts += [v[DH * h:DH * h + DH], tail]
        vt[:, c0:c0 + n] = _pk(jnp.concatenate(parts, axis=0).astype(BF16))
        gt[:, c0:c0 + n] = jnp.broadcast_to(glogit, (8, n))
        return lane_tile_max(jnp.max(jnp.abs(v).reshape(D // 8, 8, n), axis=0))

    def proj_block(c0, n):
        qkv = _dot(_upk(lhs_all[...]), xs[:, c0:c0 + n])
        return (proj_q(c0, n, qkv[0:D]), proj_k(c0, n, qkv[D:2 * D]),
                proj_v(c0, n, qkv[2 * D:3 * D], qkv[3 * D:3 * D + 1]))

    def dft_d_block(c0, n):
        cols = slice(c0, c0 + n)
        xf = xs[:, cols].astype(F32)
        xj = [xf[E8 * j:E8 * j + E8] for j in range(8)]
        a = [xj[j] + xj[j + 4] for j in range(4)]
        b = [xj[j] - xj[j + 4] for j in range(4)]
        ae, ao = a[0] + a[2], a[1] + a[3]
        p, q = (b[1] - b[3]) * _RS2, (b[1] + b[3]) * _RS2
        ops = [(ae + ao, ae - ao), (a[0] - a[2], a[3] - a[1]), (b[0] + p, -(b[2] + q)), (b[0] - p, b[2] - q)]
        for t in range(4):
            y = jnp.concatenate(ops[t], axis=0).astype(BF16)
            lhs = _upk(ff[_ROW0[t] // 2:_ROW0[t + 1] // 2, :])[:, 0:Q4]
            x1t[_ROW0[t]:_ROW0[t + 1], cols] = _dot(lhs, y)

    x_copy(0).wait()
    in_copies[1].wait()
    for c in w_copies[0:4]:
        c.wait()
    for c in w_copies[4:7]:
        c.start()
    prep_w(0, 4, wait=False)
    dft_d_block(0, QB)
    xb0 = xs[:, 0:QB]
    for c in w_copies[4:6]:
        c.wait()
    for c in w_copies[7:]:
        c.start()
    in_copies[0].start()
    w_copies[6].wait()
    prep_w(4, 7, wait=False)
    amax0 = proj_q(0, QB, _dot(_upk(lhs_all[0:D // 2, :]), xb0))
    for b in range(1, NQB):
        x_copy(b).start()
    for c in w_copies[7:]:
        c.wait()
    in_copies[0].wait()
    prep_w(7, 11, wait=False)
    gate16 = jnp.concatenate([gate_s[...].reshape(1, D).astype(F32), jnp.zeros((15, D), F32)], axis=0)
    lhs_all[3 * D // 2:3 * D // 2 + 8, :] = _pk(gate16.astype(BF16))
    kmax0 = proj_k(0, QB, _dot(_upk(lhs_all[D // 2:D, :]), xb0))
    vg = _dot(_upk(lhs_all[D:3 * D // 2 + 8, :]), xb0)
    st = [(amax0, kmax0, proj_v(0, QB, vg[0:D], vg[D:D + 1]))]
    for c in in_copies[2:]:
        c.start()
    for b in range(1, NQB):
        x_copy(b).wait()
    st.append(proj_block(QB, QB))
    st.append(proj_block(2 * QB, QB))
    dft_d_block(QB, QB)
    st.append(proj_block(3 * QB, QB))
    dft_d_block(2 * QB, QB)
    dft_d_block(3 * QB, QB)
    amax, kmax, vmax = [jnp.maximum(jnp.maximum(a, b), jnp.maximum(c, d)) for a, b, c, d in zip(*st)]

    kcol = jnp.max(kmax, axis=1, keepdims=True)
    prod = (amax * kcol).astype(BF16)
    hh = lax.broadcasted_iota(jnp.int32, (H, D), 0)
    jj = lax.broadcasted_iota(jnp.int32, (H, D), 1)
    ind = jnp.where((jj >= DH * hh) & (jj < DH * hh + DH), 1.0, 0.0).astype(BF16)
    bound = jnp.max(_dot(ind, prod)) * 1.03
    vmax = jnp.max(vmax)
    safe = jnp.logical_and(bound <= _SAFE_SCORE, jnp.logical_and(vmax <= _V_HI, vmax >= _V_LO))

    for c in in_copies[2:]:
        c.wait()

    def late_prep():
        for a, w_s in enumerate((wr_s, wi_s)):
            last = jnp.concatenate([w_s[DF - 1:DF, :].astype(F32), jnp.zeros((63, S), F32)], axis=0).astype(BF16)
            for j in range(16):
                w32[a, j, 0:112, :] = _pk(w_s[0:DF - 1, 128 * j:128 * j + 128])
                w32[a, j, 112:144, :] = _pk(last[:, 128 * j:128 * j + 128])
        wo = wo_s[...].astype(F32)
        parts = []
        for h in range(H):
            parts += [wo[DH * h:DH * h + DH], jnp.zeros((4, D), F32)]
        wot[...] = _pk(jnp.concatenate(parts, axis=0).astype(BF16).T)

    def tw_pair(k1):
        return tw[8 * k1:8 * k1 + 8, :], tw[128 + 8 * k1:128 + 8 * k1 + 8, :]

    lane = lax.broadcasted_iota(jnp.int32, (8, 128), 1)

    def butterfly(z, h):
        sig = jnp.where((lane & h) == 0, 1.0, -1.0)
        if h == 64:
            return tuple(pltpu.roll(c, 64, 1) + sig * c for c in z)
        low = (lane & h) == 0
        return tuple(jnp.where(low, pltpu.roll(c, 128 - h, 1), pltpu.roll(c, h, 1)) + sig * c for c in z)

    def rot_quarter(z, h, sign):
        m = jnp.logical_and((lane & h) != 0, (lane & (h // 2)) != 0)
        re, im = z
        if sign < 0:
            return jnp.where(m, im, re), jnp.where(m, -re, im)
        return jnp.where(m, -im, re), jnp.where(m, re, im)

    def lane_tw(z, i, sign):
        c, s = tw[256 + 16 * i:264 + 16 * i, :], tw[264 + 16 * i:272 + 16 * i, :]
        re, im = z
        if sign < 0:
            return re * c + im * s, im * c - re * s
        return re * c - im * s, im * c + re * s

    def lane_fft(zs):
        for i, h in enumerate((64, 16, 4)):
            zs = [butterfly(z, h) for z in zs]
            zs = [rot_quarter(z, h, -1) for z in zs]
            zs = [butterfly(z, h // 2) for z in zs]
            zs = [lane_tw(z, i, -1) for z in zs]
        return [butterfly(z, 1) for z in zs]

    def lane_ifft(zs):
        zs = [butterfly(z, 1) for z in zs]
        for i, h in reversed(list(enumerate((64, 16, 4)))):
            zs = [lane_tw(z, i, +1) for z in zs]
            zs = [butterfly(z, h // 2) for z in zs]
            zs = [rot_quarter(z, h, +1) for z in zs]
            zs = [butterfly(z, h) for z in zs]
        return zs

    def filter_rows(a, pa, pb, shift):
        m10 = (lane & 80) == 64
        m01 = (lane & 80) == 16
        top4 = lax.broadcasted_iota(jnp.int32, (8, 128), 0) < 4
        v = []
        for j in range(16):
            w = jnp.where(top4, w32[a, j, pl.ds(pa, 8, stride=4), :], w32[a, j, pl.ds(pb, 8, stride=4), :])
            w = pltpu.bitcast((w << shift) & jnp.uint32(0xFFFF0000), F32)
            v.append(jnp.where(m10, pltpu.roll(w, 48, 1), jnp.where(m01, pltpu.roll(w, 80, 1), w)))
        for i in range(4):
            t, d = 1 << i, 8 >> i
            low = (lane & d) == 0
            for j in range(16):
                if j & t == 0:
                    lo, hi = v[j], v[j + t]
                    v[j] = jnp.where(low, lo, pltpu.roll(hi, d, 1))
                    v[j + t] = jnp.where(low, pltpu.roll(lo, 128 - d, 1), hi)
        return [v[int(format(k1, '04b')[::-1], 2)] for k1 in range(16)]

    def spectral_group(gi):
        blk = x1t[pl.ds(pl.multiple_of(gi * 16, 16), 16), :]
        xin = [(blk[0:8, 128 * a:128 * a + 128], blk[8:16, 128 * a:128 * a + 128]) for a in range(16)]
        y = _dft16(xin, -1)
        t1, t2, t3 = gi >= 8, gi >= 15, gi >= 22
        r = jnp.where(t3, 3, jnp.where(t2, 1, jnp.where(t1, 2, 0)))
        rc = jnp.where(t3, 5, jnp.where(t2, 7, jnp.where(t1, 6, 4)))
        g = gi - jnp.where(t3, 22, jnp.where(t2, 15, jnp.where(t1, 8, 0)))
        fa = jnp.where(g < 4, r + 64 * g, jnp.where(g < 7, rc + 64 * (g - 4), D // 2))
        fb = jnp.where(g == 3, rc + 192, fa + 32)
        pa, pb = fa // 2, fb // 2 - 16
        shift = jnp.asarray(16 - 16 * (r % 2)).astype(U32)
        wr_ = filter_rows(0, pa, pb, shift)
        wi_ = filter_rows(1, pa, pb, shift)
        zs = []
        for k1 in range(16):
            re, im = y[k1]
            if k1:
                c, s = tw_pair(k1)
                re, im = re * c + im * s, im * c - re * s
            zs.append((re, im))
        zs = lane_fft(zs)
        zs = [(re * wr_[k1] - im * wi_[k1], re * wi_[k1] + im * wr_[k1]) for k1, (re, im) in enumerate(zs)]
        zs = lane_ifft(zs)
        zin = []
        for k1 in range(16):
            re, im = zs[k1]
            if k1:
                c, s = tw_pair(k1)
                re, im = re * c - im * s, im * c + re * s
            zin.append((re, im))
        z = _dft16(zin, +1)
        top = jnp.concatenate([z[a][0] for a in range(16)], axis=1)
        bot = jnp.concatenate([z[a][1] for a in range(16)], axis=1)
        zt[pl.ds(pl.multiple_of(gi * 8, 8), 8), :] = _pk(jnp.concatenate([top, bot], axis=0).astype(BF16))

    def scores(n):
        h = n // NAQ
        t = h // 4
        i = h % 4
        cols = pl.ds(pl.multiple_of((n % NAQ) * AW, AW), AW)
        q32 = qt[pl.ds(pl.multiple_of(56 * t, 8), 56), cols]
        rr = lax.broadcasted_iota(jnp.int32, (56, AW), 0)
        q32 = jnp.where((rr >= 14 * i) & (rr < 14 * i + 14), q32, jnp.uint32(0))
        qm = _upk(jnp.concatenate([q32, jnp.zeros((8, AW), U32)], axis=0))
        kt = _upk(ks[:, pl.ds(pl.multiple_of(128 * t, 128), 128)])
        return _dot(kt, qm)

    def qk_exp(n, p_ref):
        p_ref[...] = _pk(jnp.exp2(scores(n)).astype(BF16))

    def pv(n, p_ref):
        h = n // NAQ
        rows = pl.ds(pl.multiple_of(16 * h, 16), 16)
        o = _dot(_upk(vt[rows, :]), _upk(p_ref[...]))
        o = o * (1.0 / o[DH:DH + 1, :])
        ot[rows, pl.ds(pl.multiple_of((n % NAQ) * AW, AW), AW)] = _pk(o.astype(BF16))

    @pl.when(safe)
    def _fast():
        late_prep()
        qk_exp(0, p0)
        qk_exp(1, p1)

        def body(j, carry):
            for m in range(GPI):
                spectral_group(jnp.minimum(GPI * j + m, NG - 1))
            pv(2 * j, p0)
            qk_exp(2 * j + 2, p0)
            pv(2 * j + 1, p1)
            qk_exp(2 * j + 3, p1)
            return carry

        lax.fori_loop(0, NIT, body, 0)
        pv(NBLK - 2, p0)
        pv(NBLK - 1, p1)
        for gi in range(NIT * GPI, NG):
            spectral_group(gi)

    @pl.when(jnp.logical_not(safe))
    def _slow():
        late_prep()

        def body(n, carry):
            sbuf[...] = scores(n)
            m = jnp.max(jnp.max(sbuf[...].reshape(S // 8, 8, AW), axis=0), axis=0, keepdims=True)
            p0[...] = _pk(jnp.exp2(sbuf[...] - m).astype(BF16))
            pv(n, p0)
            return carry

        lax.fori_loop(0, NBLK, body, 0)

        def fbody(gi, carry):
            spectral_group(gi)
            return carry

        lax.fori_loop(0, NG, fbody, 0)

    out_blocks = [(0, 512), (512, 512), (1024, 512), (1536, 384), (1920, 128)]

    def out_copy(b):
        c = pl.ds(*out_blocks[b])
        return pltpu.make_async_copy(outb.at[:, c], out_hbm.at[:, c], sem_out.at[b])

    for b, (c0, n) in enumerate(out_blocks):
        cols = slice(c0, c0 + n)
        tt = []
        for t in range(4):
            k = _ROW0[t + 1] - _ROW0[t]
            r_ = _dot(_upk(gg[Q4 * t // 2:Q4 * (t + 1) // 2, :])[:, 0:k], _upk(zt[_ROW0[t] // 2:_ROW0[t + 1] // 2, cols]))
            tt.append((r_[0:E8], r_[E8:2 * E8]))
        (t0, t4), (a2, b2), (a1, b1), (a3, b3) = tt
        ee, eo = t0 + t4, t0 - t4
        m1, p1_ = (a1 - b1) * _RS2, (a1 + b1) * _RS2
        m3, p3 = (a3 - b3) * _RS2, (a3 + b3) * _RS2
        u0, u2, u1, u3 = ee + a2, ee - a2, eo - b2, eo + b2
        w0, w2, w1, w3 = a1 + a3, b3 - b1, m1 - p3, m3 - p1_
        yt = jnp.concatenate([u0 + w0, u1 + w1, u2 + w2, u3 + w3, u0 - w0, u1 - w1, u2 - w2, u3 - w3], axis=0)
        g = jax.nn.sigmoid(gt[0:1, cols])
        yt = (1.0 - g) * yt
        at = _dot(_upk(wot[...]), _upk(ot[:, cols]))
        outb[:, cols] = (g * at + yt).astype(BF16)
        out_copy(b).start()
    for b in range(len(out_blocks)):
        out_copy(b).wait()


@jax.jit
def pallas_gated_mix__softmax_full_mha__spectral_gfnet__prompt_kernel(
    A_x: jax.Array,
    A_wqkv: jax.Array,
    A_wo: jax.Array,
    B_x: jax.Array,
    B_w_r: jax.Array,
    B_w_i: jax.Array,
    gate_w: jax.Array,
):
    del B_x
    ff_np, gg_np, tw_np = _tables()
    any_spec = pl.BlockSpec(memory_space=pltpu.HBM)
    scratch = [
        pltpu.VMEM((D, S), BF16),
        pltpu.VMEM((D, 3 * D), BF16),
        pltpu.VMEM((D, D), BF16),
        pltpu.VMEM((DF, S), BF16),
        pltpu.VMEM((DF, S), BF16),
        pltpu.VMEM((D,), BF16),
        pltpu.VMEM(ff_np.shape, U32),
        pltpu.VMEM(gg_np.shape, U32),
        pltpu.VMEM(tw_np.shape, F32),
        pltpu.VMEM((3 * D // 2 + 8, D), U32),
        pltpu.VMEM((D // 2, 512), U32),
        pltpu.VMEM((S // 2, 512), U32),
        pltpu.VMEM((D // 2, S), U32),
        pltpu.VMEM((256, S), U32),
        pltpu.VMEM((256, S), U32),
        pltpu.VMEM((8, S), F32),
        pltpu.VMEM((S // 2, AW), U32),
        pltpu.VMEM((S // 2, AW), U32),
        pltpu.VMEM((NROW, S), F32),
        pltpu.VMEM((2, 16, 144, 128), U32),
        pltpu.VMEM((NROW // 2, S), U32),
        pltpu.VMEM((D, S), BF16),
        pltpu.VMEM((S, AW), F32),
        pltpu.SemaphoreType.DMA((NQB,)),
        pltpu.SemaphoreType.DMA((11,)),
        pltpu.SemaphoreType.DMA((7,)),
        pltpu.SemaphoreType.DMA((5,)),
    ]
    out = pl.pallas_call(
        _kernel,
        out_shape=jax.ShapeDtypeStruct((D, S), BF16),
        in_specs=[any_spec] * 9,
        out_specs=any_spec,
        scratch_shapes=scratch,
        compiler_params=pltpu.CompilerParams(vmem_limit_bytes=100 * 1024 * 1024),
    )(A_x.reshape(S, D).T, A_wqkv, A_wo, B_w_r.T, B_w_i.T, gate_w,
      jnp.asarray(ff_np), jnp.asarray(gg_np), jnp.asarray(tw_np))
    return out.T.reshape(1, S, D)
```
